```python
import jax
import jax.numpy as jnp

def _softmax(x, axis=-1):
    return jax.nn.softmax(x, axis=axis)
def _gelu(x):
    return jax.nn.gelu(x, approximate=True)
def _silu(x):
    return jax.nn.silu(x)
def _sigmoid(x):
    return jax.nn.sigmoid(x)
def _layernorm(x, axis=-1, eps=1e-5):
    m = jnp.mean(x, axis=axis, keepdims=True)
    v = jnp.var(x, axis=axis, keepdims=True)
    return (x - m) / jnp.sqrt(v + eps)
def _scatter_add(tgt, idx, src, axis=0):
    return tgt.at[idx].add(src)
def _segment_sum(src, seg, n):
    return jax.ops.segment_sum(src, seg, n)
class _Rng:
    def __init__(self, key):
        self._k = key
    def _next(self):
        self._k, sub = jax.random.split(self._k)
        return sub
    def normal(self, shape):
        return jax.random.normal(self._next(), shape, dtype=jnp.bfloat16)
    def randint(self, lo, hi, shape):
        return jax.random.randint(self._next(), shape, lo, hi, dtype=jnp.int32)
    def uniform(self, shape, lo=0.0, hi=1.0):
        return jax.random.uniform(self._next(), shape, jnp.bfloat16, lo, hi)
    def permutation(self, n):
        return jax.random.permutation(self._next(), n)


kernel_name = 'interleave_layers__softmax_full_mha__ssm_conv_h3__prompt'

def setup_inputs():
    _rng = _Rng(jax.random.key(int.from_bytes(__import__("os").urandom(4), "little")))
    _w = (lambda a: (lambda t: t.astype(jnp.bfloat16) if jnp.issubdtype(t.dtype, jnp.floating) else t)(jnp.asarray(a)))
    def _A_setup():
        B, S, D = 1, 2048, 1024
        return {
            "x": _w((lambda *s: _rng.normal(s) * 0.05)(B, S, D)),
            "wqkv": _w((lambda *s: _rng.normal(s) * 0.05)(D, 3 * D)),
            "wo": _w((lambda *s: _rng.normal(s) * 0.05)(D, D)),
        }
    _A_in = _A_setup()

    def _B_setup():
        B, S, D = 1, 2048, 1024
        ks = 4
        return {
            "q": _w((lambda *s: _rng.normal(s) * 0.05)(B, S, D)),
            "k": _w((lambda *s: _rng.normal(s) * 0.05)(B, S, D)),
            "v": _w((lambda *s: _rng.normal(s) * 0.05)(B, S, D)),
            "shift_k": _w((lambda *s: _rng.normal(s) * 0.05)(D, ks) * 0.5),
            "ssm_k": _w((lambda *s: _rng.normal(s) * 0.05)(D, S) * (1.0 / S ** 0.5)),
            "ssm_D": _w((lambda *s: _rng.normal(s) * 0.05)(D)),
        }
    _B_in = _B_setup()

    return {
        "A_x": _A_in["x"],
        "A_wqkv": _A_in["wqkv"],
        "A_wo": _A_in["wo"],
        "B_q": _B_in["q"],
        "B_k": _B_in["k"],
        "B_v": _B_in["v"],
        "B_shift_k": _B_in["shift_k"],
        "B_ssm_k": _B_in["ssm_k"],
        "B_ssm_D": _B_in["ssm_D"],
    }

def reference(A_x, A_wqkv, A_wo, B_q, B_k, B_v, B_shift_k, B_ssm_k, B_ssm_D):
    def _A_ref(x, wqkv, wo):
        B, S, D = x.shape
        H = 32; Dh = D // H
        qkv = (lambda x, *d: x.transpose(*d))((x @ wqkv).reshape(B, S, 3, H, Dh), 2, 0, 3, 1, 4)
        q, k, v = qkv[0], qkv[1], qkv[2]
        scale = Dh ** -0.5
        scores = jnp.einsum("bhqd,bhkd->bhqk", q, k) * scale
        p = _softmax(scores, axis=-1)
        o = jnp.einsum("bhqk,bhkd->bhqd", p, v)
        return (lambda x, *d: x.transpose(*d))(o, 0, 2, 1, 3).reshape(B, S, D) @ wo

    def _B_ref(q, k, v, shift_k, ssm_k, ssm_D):
        B, S, D = q.shape
        ks = shift_k.shape[-1]
        k_pad = jnp.pad(k, ((0, 0), (ks - 1, 0), (0, 0)))
        k_shift = jnp.zeros_like(k)
        for t in range(ks):
            k_shift = k_shift + k_pad[:, t:t + S, :] * shift_k[:, ks - 1 - t][None, None, :]
        kv = k_shift * v
        L = 2 * S
        kv_pad = jnp.pad(kv, ((0, 0), (0, S), (0, 0)))
        kf_pad = jnp.pad(ssm_k, ((0, 0), (0, S)))
        kv_f = (lambda x, axes=(-2,-1): jnp.fft.rfft2(x.astype(jnp.float32), axes=axes))(kv_pad[:, None, :, :], axes=(1, 2))
        kf_f = (lambda x, axes=(-2,-1): jnp.fft.rfft2(x.astype(jnp.float32), axes=axes))(kf_pad[:, None, :], axes=(1, 2))
        kf_f = (lambda x, *d: x.transpose(*d))(kf_f, 1, 2, 0)
        y_f = kv_f * kf_f[None, :, :, :]
        y = (lambda x, s, axes=(-2,-1): jnp.fft.irfft2(x, s=s, axes=axes).astype(jnp.bfloat16))(y_f, (1, L), axes=(1, 2))[:, 0, :S, :]
        y = y + kv * ssm_D[None, None, :]
        return q * y

    x = A_x
    x = x + _A_ref(_layernorm(x, axis=-1), A_wqkv, A_wo)
    x = x + _B_ref(_layernorm(x, axis=-1), B_k, B_v, B_shift_k, B_ssm_k, B_ssm_D)
    x = x + _A_ref(_layernorm(x, axis=-1), A_wqkv, A_wo)
    x = x + _B_ref(_layernorm(x, axis=-1), B_k, B_v, B_shift_k, B_ssm_k, B_ssm_D)
    return x
```

```python
import math
import numpy as np
import jax
import jax.numpy as jnp
from jax import lax
import jax.experimental.pallas as pl
import jax.experimental.pallas.tpu as pltpu

S, D, H, DH = 2048, 1024, 32, 32
TQ = 256
NT = S // TQ
CK = 128
BL = 128
NB = S // BL
F32, BF16 = jnp.float32, jnp.bfloat16


def _dft_mats():
    n = 2 * BL
    k = np.arange(BL)[:, None]
    t = np.arange(BL)[None, :]
    f = np.concatenate([np.cos(2 * np.pi * k * t / n), -np.sin(2 * np.pi * k * t / n)], 0)
    f[BL] = np.cos(np.pi * np.arange(BL))
    tt = np.arange(n)[:, None]
    kk = np.arange(BL)[None, :]
    g = np.concatenate([2 * np.cos(2 * np.pi * kk * tt / n), -2 * np.sin(2 * np.pi * kk * tt / n)], 1)
    g[:, 0] = 1.0
    g[:, BL] = np.cos(np.pi * np.arange(n))
    return f.astype(np.float32), (g / n).astype(np.float32)


def _ln(x):
    m = jnp.mean(x, axis=-1, keepdims=True)
    d = x - m
    v = jnp.mean(d * d, axis=-1, keepdims=True)
    return d * lax.rsqrt(v + 1e-5)


def _kernel(x_hbm, wqkv_hbm, wo_hbm, k_hbm, v_hbm, shk_ref, ssk_hbm, ssd_ref, f_ref, g_ref,
            out_ref,
            xin, wqkv, wo, kb, vb, skb, xs, y_s, k3, qt, vt, ot,
            s0, s1, s2, s3, m0, m1, m2, m3, a_s, b_s, c_s, sems):
    srcs = (x_hbm, wqkv_hbm, k_hbm, v_hbm, ssk_hbm, wo_hbm)
    dsts = (xin, wqkv, kb, vb, skb, wo)
    cps = [pltpu.make_async_copy(a, b, sems.at[i]) for i, (a, b) in enumerate(zip(srcs, dsts))]
    for c in cps:
        c.start()

    def rows(t):
        return pl.ds(pl.multiple_of(t * TQ, TQ), TQ)

    def project(t, x):
        xn = _ln(x).astype(BF16)
        q = jnp.dot(xn, wqkv[:, 0:D], preferred_element_type=F32)
        qt[t] = (q * (DH ** -0.5 * math.log2(math.e))).T.astype(BF16)
        k = jnp.dot(xn, wqkv[:, D:2 * D], preferred_element_type=F32).astype(BF16)
        for h in range(H):
            k3[h, rows(t), :] = k[:, h * DH:(h + 1) * DH]
        v = jnp.dot(xn, wqkv[:, 2 * D:3 * D], preferred_element_type=F32)
        vt[:, rows(t)] = v.T.astype(BF16)

    NU = H * NT

    def hs(h):
        return pl.ds(pl.multiple_of(h * DH, DH), DH)

    def qk(i, s_ref, m_ref):
        h, t = i // NT, i % NT
        w = qt[t, hs(h), :]
        mm = None
        for c in range(S // CK):
            s = jnp.dot(k3[h, pl.ds(c * CK, CK), :], w, preferred_element_type=F32)
            s_ref[pl.ds(c * CK, CK), :] = s
            mc = jnp.max(s.reshape(CK // 8, 8, TQ), axis=0)
            mm = mc if mm is None else jnp.maximum(mm, mc)
        m_ref[...] = jnp.broadcast_to(jnp.max(mm, axis=0, keepdims=True), (8, TQ))

    def both(i, sa, ma, sb, mb):
        i1 = jnp.minimum(i + 2, NU - 1)
        h1, t1 = i1 // NT, i1 % NT
        w = qt[t1, hs(h1), :]
        h, t = i // NT, i % NT
        m = ma[...]
        mm = acc = l = None
        for c in range(S // CK):
            ck = pl.ds(c * CK, CK)
            s = jnp.dot(k3[h1, ck, :], w, preferred_element_type=F32)
            sb[ck, :] = s
            mc = jnp.max(s.reshape(CK // 8, 8, TQ), axis=0)
            mm = mc if mm is None else jnp.maximum(mm, mc)
            p = jnp.exp2(sa[ck, :].reshape(CK // 8, 8, TQ) - m[None])
            lc = jnp.sum(p, axis=0)
            l = lc if l is None else l + lc
            a = jnp.dot(vt[hs(h), ck], p.reshape(CK, TQ).astype(BF16), preferred_element_type=F32)
            acc = a if acc is None else acc + a
        mb[...] = jnp.broadcast_to(jnp.max(mm, axis=0, keepdims=True), (8, TQ))
        l = jnp.sum(l, axis=0, keepdims=True)
        ot[t, hs(h), :] = acc * (1.0 / l)

    def attention():
        bufs = [(s0, m0), (s1, m1), (s2, m2), (s3, m3)]
        qk(0, s0, m0)
        qk(1, s1, m1)

        def body(j, c):
            for u in range(4):
                both(4 * j + u, *bufs[u], *bufs[(u + 2) % 4])
            return c
        lax.fori_loop(0, NU // 4, body, 0)

    def mix(t):
        o = ot[t].T.astype(BF16)
        x1 = xs[rows(t), :] + jnp.dot(o, wo[...], preferred_element_type=F32)
        return x1 + _ln(x1) * y_s[rows(t), :]

    def ssm(cb, carry):
        ls = pl.ds(pl.multiple_of(cb * 128, 128), 128)
        k = kb[:, ls].astype(F32)
        row = lax.broadcasted_iota(jnp.int32, (S, 128), 0)
        ks = k * shk_ref[0:1, ls]
        for d in range(1, 4):
            ks = ks + jnp.where(row >= d, pltpu.roll(k, d, 0), 0.0) * shk_ref[d:d + 1, ls]
        kv = ks * vb[:, ls].astype(F32)
        kvb = kv.astype(BF16)
        xa = jnp.concatenate([kvb[j * BL:(j + 1) * BL] for j in range(NB)], axis=1)
        a_s[...] = jnp.dot(f_ref[...], xa, preferred_element_type=F32)
        fk = skb[ls, :].astype(F32)
        xb = jnp.concatenate([fk[:, j * BL:(j + 1) * BL].T for j in range(NB)], axis=1).astype(BF16)
        b_s[...] = jnp.dot(f_ref[...], xb, preferred_element_type=F32)

        def prod(r, c):
            re = pl.ds(pl.multiple_of(r * 8, 8), 8)
            im = pl.ds(pl.multiple_of(BL + r * 8, 8), 8)
            z = (lax.broadcasted_iota(jnp.int32, (8, 128), 0) + r * 8) == 0
            A, B = [], []
            for j in range(NB):
                cs = slice(j * 128, (j + 1) * 128)
                ar, ai, br, bi = a_s[re, cs], a_s[im, cs], b_s[re, cs], b_s[im, cs]
                A.append((ar, ai, jnp.where(z, 0.0, ar), jnp.where(z, 0.0, ai)))
                B.append((br, bi, jnp.where(z, bi, br)))
            for n in range(NB):
                yr = yi = None
                for j in range(n + 1):
                    ar, ai, arz, aiz = A[j]
                    br, bi, brz = B[n - j]
                    pr = ar * br - aiz * bi
                    pi = arz * bi + ai * brz
                    yr = pr if yr is None else yr + pr
                    yi = pi if yi is None else yi + pi
                c_s[re, n * 128:(n + 1) * 128] = yr
                c_s[im, n * 128:(n + 1) * 128] = yi
            return c
        lax.fori_loop(0, BL // 8, prod, 0)
        full = jnp.dot(g_ref[...], c_s[...].astype(BF16), preferred_element_type=F32)
        dv = ssd_ref[0:1, ls]
        for n in range(NB):
            yb = full[0:BL, n * 128:(n + 1) * 128]
            if n:
                yb = yb + full[BL:, (n - 1) * 128:n * 128]
            y_s[pl.ds(n * BL, BL), ls] = yb + kv[n * BL:(n + 1) * BL] * dv
        return carry

    cps[0].wait()
    cps[1].wait()

    def first(t, c):
        x = xin[rows(t), :].astype(F32)
        xs[rows(t), :] = x
        project(t, x)
        return c
    lax.fori_loop(0, NT, first, 0)
    for c in cps[2:]:
        c.wait()
    lax.fori_loop(0, D // 128, ssm, 0)

    def layer(li, c):
        attention()

        @pl.when(li == 0)
        def _():
            def mid(t, c2):
                x2 = mix(t)
                xs[rows(t), :] = x2
                return c2
            lax.fori_loop(0, NT, mid, 0)
            lax.fori_loop(0, NT, lambda t, c2: (project(t, xs[rows(t), :]), c2)[1], 0)
        return c
    lax.fori_loop(0, 2, layer, 0)

    def last(t, c):
        out_ref[rows(t), :] = mix(t).astype(BF16)
        return c
    lax.fori_loop(0, NT, last, 0)


@jax.jit
def pallas_interleave_layers__softmax_full_mha__ssm_conv_h3__prompt_kernel(
    A_x, A_wqkv, A_wo, B_q, B_k, B_v, B_shift_k, B_ssm_k, B_ssm_D,
):
    del B_q
    f, g = _dft_mats()
    anyspec = pl.BlockSpec(memory_space=pl.ANY)
    vm = pl.BlockSpec(memory_space=pltpu.VMEM)
    scratch = [
        pltpu.VMEM((S, D), BF16), pltpu.VMEM((D, 3 * D), BF16), pltpu.VMEM((D, D), BF16),
        pltpu.VMEM((S, D), BF16), pltpu.VMEM((S, D), BF16), pltpu.VMEM((D, S), BF16),
        pltpu.VMEM((S, D), F32), pltpu.VMEM((S, D), F32),
        pltpu.VMEM((H, S, DH), BF16), pltpu.VMEM((NT, D, TQ), BF16), pltpu.VMEM((D, S), BF16),
        pltpu.VMEM((NT, D, TQ), F32),
    ] + [pltpu.VMEM((S, TQ), F32)] * 4 + [pltpu.VMEM((8, TQ), F32)] * 4 \
      + [pltpu.VMEM((2 * BL, S), F32)] * 3 + [pltpu.SemaphoreType.DMA((6,))]
    out = pl.pallas_call(
        _kernel,
        out_shape=jax.ShapeDtypeStruct((S, D), BF16),
        in_specs=[anyspec] * 5 + [vm, anyspec, vm, vm, vm],
        out_specs=vm,
        scratch_shapes=scratch,
        compiler_params=pltpu.CompilerParams(vmem_limit_bytes=124 * 1024 * 1024),
    )(A_x.reshape(S, D), A_wqkv, A_wo, B_k.reshape(S, D), B_v.reshape(S, D),
      B_shift_k.T.astype(F32), B_ssm_k, B_ssm_D.reshape(1, D).astype(F32),
      jnp.asarray(f, BF16), jnp.asarray(g, BF16))
    return out.reshape(1, S, D)
```
